```python
import os as _os
_os.environ.setdefault("JAX_PLATFORMS", "cpu")
import jax
import jax.numpy as jnp

def _softmax(x, axis=-1):
    return jax.nn.softmax(x, axis=axis)
def _gelu(x):
    return jax.nn.gelu(x, approximate=True)
def _silu(x):
    return jax.nn.silu(x)
def _sigmoid(x):
    return jax.nn.sigmoid(x)
def _layernorm(x, axis=-1, eps=1e-5):
    m = jnp.mean(x, axis=axis, keepdims=True)
    v = jnp.var(x, axis=axis, keepdims=True)
    return (x - m) / jnp.sqrt(v + eps)
def _scatter_add(tgt, idx, src, axis=0):
    return tgt.at[idx].add(src)
def _segment_sum(src, seg, n):
    return jax.ops.segment_sum(src, seg, n)
class _Rng:
    def __init__(self, key):
        self._k = key
    def _next(self):
        self._k, sub = jax.random.split(self._k)
        return sub
    def normal(self, shape):
        return jax.random.normal(self._next(), shape, dtype=jnp.bfloat16)
    def randint(self, lo, hi, shape):
        return jax.random.randint(self._next(), shape, lo, hi, dtype=jnp.int32)
    def uniform(self, shape, lo=0.0, hi=1.0):
        return jax.random.uniform(self._next(), shape, jnp.bfloat16, lo, hi)
    def permutation(self, n):
        return jax.random.permutation(self._next(), n)


kernel_name = 'parallel_sum__ssm_conv_s5__glu_gated_swiglu__prompt'

def setup_inputs():
    _rng = _Rng(jax.random.key(int.from_bytes(__import__("os").urandom(4), "little")))
    _w = (lambda a: (lambda t: t.astype(jnp.bfloat16) if jnp.issubdtype(t.dtype, jnp.floating) else t)(jnp.asarray(a)))
    def _A_setup():
        B, S, D = 1, 2048, 640
        P = D
        Lambda_re = -0.5 * jnp.exp((lambda *s: _rng.normal(s) * 0.4)(P))
        Lambda_im = (lambda *s: _rng.normal(s) * 0.4)(P) * 1.0
        B_re = (lambda *s: _rng.normal(s) * 0.4)(P, D) * (D ** -0.5)
        B_im = (lambda *s: _rng.normal(s) * 0.4)(P, D) * (D ** -0.5)
        C_re = (lambda *s: _rng.normal(s) * 0.4)(D, P) * (P ** -0.5)
        C_im = (lambda *s: _rng.normal(s) * 0.4)(D, P) * (P ** -0.5)
        log_dt = (lambda *s: _rng.normal(s) * 0.4)(P) * 0.3 - 2.0
        Dskip = (lambda *s: _rng.normal(s) * 0.4)(D)
        return {
            "x": _w((lambda *s: _rng.normal(s) * 0.05)(B, S, D)),
            "Lambda_re": _w(Lambda_re),
            "Lambda_im": _w(Lambda_im),
            "B_re": _w(B_re),
            "B_im": _w(B_im),
            "C_re": _w(C_re),
            "C_im": _w(C_im),
            "log_dt": _w(log_dt),
            "Dskip": _w(Dskip),
        }
    _A_in = _A_setup()

    def _B_setup():
        B, S, D, F = 1, 2048, 640, 1728
        return {
            "x": _w((lambda *s: _rng.normal(s) * 0.05)(B, S, D)),
            "w1": _w((lambda *s: _rng.normal(s) * 0.1)(D, F) * (2.0 / D) ** 0.5),
            "w3": _w((lambda *s: _rng.normal(s) * 0.1)(D, F) * (2.0 / D) ** 0.5),
            "w2": _w((lambda *s: _rng.normal(s) * 0.1)(F, D) * (2.0 / F) ** 0.5),
        }
    _B_in = _B_setup()

    return {
        "A_x": _A_in["x"],
        "A_Lambda_re": _A_in["Lambda_re"],
        "A_Lambda_im": _A_in["Lambda_im"],
        "A_B_re": _A_in["B_re"],
        "A_B_im": _A_in["B_im"],
        "A_C_re": _A_in["C_re"],
        "A_C_im": _A_in["C_im"],
        "A_log_dt": _A_in["log_dt"],
        "A_Dskip": _A_in["Dskip"],
        "B_x": _B_in["x"],
        "B_w1": _B_in["w1"],
        "B_w3": _B_in["w3"],
        "B_w2": _B_in["w2"],
    }

def reference(A_x, A_Lambda_re, A_Lambda_im, A_B_re, A_B_im, A_C_re, A_C_im, A_log_dt, A_Dskip, B_x, B_w1, B_w3, B_w2):
    def _A_ref(x, Lambda_re, Lambda_im, B_re, B_im, C_re, C_im, log_dt, Dskip):
        Bsz, L, H = x.shape
        Lam = Lambda_re + 1j * Lambda_im
        Bmat = B_re + 1j * B_im
        Cmat = C_re + 1j * C_im
        dt = jnp.exp(log_dt)
        Lam_bar = jnp.exp(dt * Lam)
        B_bar = ((Lam_bar - 1.0) / Lam)[:, None] * Bmat
        Bu = jnp.einsum("bld,pd->blp", x + 0j, B_bar)
        h = jnp.zeros_like(Bu[:, 0, :])
        hs = []
        for t in range(L):
            h = Lam_bar[None, :] * h + Bu[:, t, :]
            hs.append(h)
        hseq = jnp.stack(hs, 1)
        y = 2.0 * jnp.einsum("blp,dp->bld", hseq, Cmat).real + x * Dskip[None, None, :]
        return y

    def _B_ref(x, w1, w3, w2):
        gate = jnp.einsum("bsd,df->bsf", x, w1)
        up = jnp.einsum("bsd,df->bsf", x, w3)
        h = _silu(gate) * up
        out = jnp.einsum("bsf,fd->bsd", h, w2)
        return out

    x = A_x
    xn = _layernorm(x, axis=-1)
    return x + _A_ref(xn, A_Lambda_re, A_Lambda_im, A_B_re, A_B_im, A_C_re, A_C_im, A_log_dt, A_Dskip) + _B_ref(xn, B_w1, B_w3, B_w2)
```

```python
import jax
import jax.numpy as jnp
from jax import lax
import jax.experimental.pallas as pl
import jax.experimental.pallas.tpu as pltpu

T = 256
FC = 256
W = 128
T0 = 512
CL = False
LE = True
LR = 16
PB = (0, 1, 2, 4)
F32 = jnp.float32
BF16 = jnp.bfloat16
NT = (((1,), (1,)), ((), ()))


def _nt(a, b):
    return lax.dot_general(a, b, NT, preferred_element_type=F32)


def _cmul(ar, ai, br, bi):
    return ar * br - ai * bi, ar * bi + ai * br


def _kernel(x_hbm, lre_hbm, lim_hbm, bre_hbm, bim_hbm, cre_hbm, cim_hbm, ldt_hbm, dsk_hbm,
            w1_hbm, w3_hbm, w2_hbm, o_hbm,
            x_v, lre_v, lim_v, ldt_v, dsk_v, b_v, c_v, w1_v, w3_v, wt_v, w2_v, o_v, r_v,
            cst, car, xn_v, hh_v, h_v, isem, osem):
    L, D = x_v.shape
    P = D
    F = w1_hbm.shape[0]
    FM = F // 128 * 128
    FT = F - FM
    NB = L // T
    chunks = [(s, min(FC, FM - s)) for s in range(0, FM, FC)]
    edges = [chunks[i][0] for i in PB] + [FM]
    pieces = [(a, b - a) for a, b in zip(edges, edges[1:])]

    copies = {}

    def add(name, src, dst):
        copies[name] = pltpu.make_async_copy(src, dst, isem.at[len(copies)])
        copies[name].start()

    add("x0", x_hbm.at[pl.ds(0, T0)], x_v.at[pl.ds(0, T0)])
    add("lre", lre_hbm, lre_v)
    add("lim", lim_hbm, lim_v)
    add("ldt", ldt_hbm, ldt_v)
    add("dsk", dsk_hbm, dsk_v)
    add("w1t", w1_hbm.at[pl.ds(FM, FT)], wt_v.at[pl.ds(0, FT)])
    add("w3t", w3_hbm.at[pl.ds(FM, FT)], wt_v.at[pl.ds(FT, FT)])
    for s, n in pieces:
        add(("w1", s), w1_hbm.at[pl.ds(s, n)], w1_v.at[pl.ds(s, n)])
        add(("w3", s), w3_hbm.at[pl.ds(s, n)], w3_v.at[pl.ds(s, n)])
    add("x1", x_hbm.at[pl.ds(T0, T)], x_v.at[pl.ds(T0, T)])
    add("bre", bre_hbm, b_v.at[pl.ds(0, P)])
    add("bim", bim_hbm, b_v.at[pl.ds(P, P)])
    add("w2", w2_hbm, w2_v.at[pl.ds(0, F)])
    add("cre", cre_hbm, c_v.at[:, pl.ds(0, P)])
    add("cim", cim_hbm, c_v.at[:, pl.ds(P, P)])
    if NB > 2:
        add("xr", x_hbm.at[pl.ds(T0 + T, L - T0 - T)], x_v.at[pl.ds(T0 + T, L - T0 - T)])
    w2_v[pl.ds(F, FT), :] = jnp.zeros((FT, D), BF16)

    def wait(*names):
        for n in names:
            copies.pop(n).wait()

    def row(ref):
        return jnp.broadcast_to(ref[...].reshape(1, P).astype(F32), (8, P))

    def consts():
        lre, lim = row(lre_v), row(lim_v)
        dt = jnp.exp(row(ldt_v)).astype(BF16).astype(F32)
        sub = lax.broadcasted_iota(jnp.int32, (8, P), 0)
        kk = (sub + 1).astype(F32)
        mag = jnp.exp(dt * lre * kk)
        ang = dt * lim * kk
        pr, pi = mag * jnp.cos(ang), mag * jnp.sin(ang)
        ar = jnp.broadcast_to(pr[0:1], (8, P))
        ai = jnp.broadcast_to(pi[0:1], (8, P))
        den = lre * lre + lim * lim
        nr = ar - 1.0
        cst[0] = 2.0 * (nr * lre + ai * lim) / den
        cst[1] = 2.0 * (ai * lre - nr * lim) / den
        for j, k in enumerate((1, 2, 4)):
            cst[2 + 2 * j] = jnp.where(sub >= k, jnp.broadcast_to(pr[k - 1:k], (8, P)), 0.0)
            cst[3 + 2 * j] = jnp.where(sub >= k, jnp.broadcast_to(-pi[k - 1:k], (8, P)), 0.0)
        cst[8] = jnp.where(sub == 0, pr, 0.0)
        cst[9] = jnp.where(sub == 0, -pi, 0.0)
        car[...] = jnp.zeros(car.shape, F32)

    def layernorm(b, n=T):
      for i in range(0, n, LR):
        rows = pl.ds(pl.multiple_of(b * T + i, LR), LR)
        x = x_v[rows, :].astype(F32)
        xc = x - jnp.mean(x, axis=-1, keepdims=True)
        v = jnp.mean(xc * xc, axis=-1, keepdims=True)
        xn = (xc * lax.rsqrt(v + 1e-5)).astype(BF16)
        xn_v[rows, :] = xn
        r_v[rows, :] = x + xn.astype(F32) * dsk_v[...].reshape(1, D).astype(F32)

    def ssm(p, xn):
        ln = pl.ds(p * W, W)
        ur = _nt(xn, b_v[pl.ds(p * W, W), :])
        ui = _nt(xn, b_v[pl.ds(P + p * W, W), :])
        k = [cst[j, :, ln] for j in range(10)]
        hr, hi = car[0, :, ln], car[1, :, ln]
        outs = []
        for r in range(xn.shape[0] // 8):
            a, b = ur[r * 8:r * 8 + 8], ui[r * 8:r * 8 + 8]
            tr, ti = _cmul(k[8], k[9], pltpu.roll(hr, 1, 0), pltpu.roll(hi, 1, 0))
            hr = (k[0] * a - k[1] * b) + tr
            hi = ti - (k[0] * b + k[1] * a)
            for j, sh in enumerate((1, 2, 4)):
                tr, ti = _cmul(k[2 + 2 * j], k[3 + 2 * j], pltpu.roll(hr, sh, 0), pltpu.roll(hi, sh, 0))
                hr, hi = hr + tr, hi + ti
            outs.append((hr, hi))
            if r % 2:
                rows = pl.ds(r * 8 - 8, 16)
                hh_v[rows, ln] = jnp.concatenate([outs[-2][0], hr], 0).astype(BF16)
                hh_v[rows, pl.ds(P + p * W, W)] = jnp.concatenate([outs[-2][1], hi], 0).astype(BF16)
        car[0, :, ln] = hr
        car[1, :, ln] = hi

    def glu(g, u):
        hg = 0.5 * g
        return (hg * jnp.tanh(hg) + hg) * u

    def block(b, first=False):
        n = T0 if first else T
        r0 = pl.multiple_of(b * T, T)
        rows, loc = pl.ds(r0, n), pl.ds(0, n)
        xn = xn_v[rows, :]
        if not first and LE:
            layernorm(jnp.minimum(b + 1, NB - 1))
        for c, (s, w) in enumerate(chunks):
            if first and ("w1", s) in copies:
                wait(("w1", s), ("w3", s))
            if not first and c < P // W:
                ssm(c, xn)
            g = _nt(xn, w1_v[pl.ds(s, w), :])
            u = _nt(xn, w3_v[pl.ds(s, w), :])
            h_v[loc, pl.ds(s, w)] = glu(g, u).astype(BF16)
        t = _nt(xn, wt_v[...])
        lane = lax.broadcasted_iota(jnp.int32, t.shape, 1)
        h_v[loc, pl.ds(FM, 2 * FT)] = jnp.where(lane < FT, glu(t, pltpu.roll(t, FT, 1)), 0.0).astype(BF16)
        if first:
            if CL:
                consts()
            wait("bre", "bim", "w2", "x1", "cre", "cim")
            layernorm(T0 // T)
            for p in range(P // W):
                ssm(p, xn)
                ln = pl.ds(p * W, W)
                o_v[rows, ln] = r_v[rows, ln] + jnp.dot(h_v[loc, :], w2_v[:, ln], preferred_element_type=F32)
            o_v[rows, :] = o_v[rows, :] + _nt(hh_v[loc, :], c_v[...])
        else:
            if not LE:
                layernorm(jnp.minimum(b + 1, NB - 1))
            acc = _nt(hh_v[loc, :], c_v[...])
            o_v[rows, :] = r_v[rows, :] + acc + jnp.dot(h_v[loc, :], w2_v[...], preferred_element_type=F32)
        pltpu.make_async_copy(o_v.at[rows], o_hbm.at[rows], osem.at[b]).start()

    wait("x0", "dsk")
    layernorm(0, T0)
    wait("lre", "lim", "ldt", "w1t", "w3t")
    if not CL:
        consts()
    block(0, first=True)
    wait("xr")
    pl.loop(T0 // T, NB)(block)
    for b, n in [(0, T0)] + [(b, T) for b in range(T0 // T, NB)]:
        rows = pl.ds(b * T, n)
        pltpu.make_async_copy(o_v.at[rows], o_hbm.at[rows], osem.at[b]).wait()


@jax.jit
def pallas_parallel_sum__ssm_conv_s5__glu_gated_swiglu__prompt_kernel(
        A_x, A_Lambda_re, A_Lambda_im, A_B_re, A_B_im, A_C_re, A_C_im, A_log_dt, A_Dskip,
        B_x, B_w1, B_w3, B_w2):
    _, L, D = A_x.shape
    P = A_Lambda_re.shape[0]
    F = B_w1.shape[1]
    FM = F // 128 * 128
    FP = FM + 2 * (F - FM)
    hbm = pl.BlockSpec(memory_space=pltpu.HBM)
    V = pltpu.VMEM
    out = pl.pallas_call(
        _kernel,
        in_specs=[hbm] * 12,
        out_specs=hbm,
        out_shape=jax.ShapeDtypeStruct((L, D), F32),
        scratch_shapes=[V((L, D), BF16), V((P,), BF16), V((P,), BF16), V((P,), BF16), V((D,), BF16),
                        V((2 * P, D), BF16), V((D, 2 * P), BF16), V((FM, D), BF16), V((FM, D), BF16),
                        V((FP - FM, D), BF16), V((FP, D), BF16), V((L, D), F32), V((L, D), F32),
                        V((10, 8, P), F32), V((2, 8, P), F32), V((L, D), BF16), V((T0, 2 * P), BF16),
                        V((T0, FP), BF16),
                        pltpu.SemaphoreType.DMA((40,)), pltpu.SemaphoreType.DMA((L // T,))],
        compiler_params=pltpu.CompilerParams(vmem_limit_bytes=100 * 1024 * 1024),
    )(A_x.reshape(L, D), A_Lambda_re, A_Lambda_im, A_B_re, A_B_im, A_C_re, A_C_im, A_log_dt, A_Dskip,
      B_w1.T, B_w3.T, B_w2)
    return out.reshape(1, L, D)
```
